```python
import os as _os
_os.environ.setdefault("JAX_PLATFORMS", "cpu")
import jax
import jax.numpy as jnp

def _softmax(x, axis=-1):
    return jax.nn.softmax(x, axis=axis)
def _gelu(x):
    return jax.nn.gelu(x, approximate=True)
def _silu(x):
    return jax.nn.silu(x)
def _sigmoid(x):
    return jax.nn.sigmoid(x)
def _layernorm(x, axis=-1, eps=1e-5):
    m = jnp.mean(x, axis=axis, keepdims=True)
    v = jnp.var(x, axis=axis, keepdims=True)
    return (x - m) / jnp.sqrt(v + eps)
def _scatter_add(tgt, idx, src, axis=0):
    return tgt.at[idx].add(src)
def _segment_sum(src, seg, n):
    return jax.ops.segment_sum(src, seg, n)
class _Rng:
    def __init__(self, key):
        self._k = key
    def _next(self):
        self._k, sub = jax.random.split(self._k)
        return sub
    def normal(self, shape):
        return jax.random.normal(self._next(), shape, dtype=jnp.bfloat16)
    def randint(self, lo, hi, shape):
        return jax.random.randint(self._next(), shape, lo, hi, dtype=jnp.int32)
    def uniform(self, shape, lo=0.0, hi=1.0):
        return jax.random.uniform(self._next(), shape, jnp.bfloat16, lo, hi)
    def permutation(self, n):
        return jax.random.permutation(self._next(), n)


kernel_name = 'gated_mix__linear_attn_block__sliding_local_dilated__prompt'

def setup_inputs():
    _rng = _Rng(jax.random.key(int.from_bytes(__import__("os").urandom(4), "little")))
    _w = (lambda a: (lambda t: t.astype(jnp.bfloat16) if jnp.issubdtype(t.dtype, jnp.floating) else t)(jnp.asarray(a)))
    def _A_setup():
        B, S, D = 1, 2048, 512
        return {
            "x": _w((lambda *s: _rng.normal(s) * 0.05)(B, S, D)),
            "wqkv": _w((lambda *s: _rng.normal(s) * 1.6)(D, 3 * D)),
            "wo": _w((lambda *s: _rng.normal(s) * 0.8)(D, D)),
        }
    _A_in = _A_setup()

    def _B_setup():
        B, S, D = 1, 2048, 512
        return {
            "x": _w((lambda *s: _rng.normal(s) * 0.05)(B, S, D)),
            "wqkv": _w((lambda *s: _rng.normal(s) * 0.8)(D, 3 * D)),
            "wo": _w((lambda *s: _rng.normal(s) * 0.05)(D, D)),
        }
    _B_in = _B_setup()

    return {
        "A_x": _A_in["x"],
        "A_wqkv": _A_in["wqkv"],
        "A_wo": _A_in["wo"],
        "B_x": _B_in["x"],
        "B_wqkv": _B_in["wqkv"],
        "B_wo": _B_in["wo"],
        "gate_w": _w((lambda *s: _rng.normal(s) * 0.05)(512) * 16.0),
    }

def reference(A_x, A_wqkv, A_wo, B_x, B_wqkv, B_wo, gate_w):
    def _A_ref(x, wqkv, wo):
        B, S, D = x.shape
        H = 32; Dh = D // H
        qkv = (lambda x, *d: x.transpose(*d))((x @ wqkv).reshape(B, S, 3, H, Dh), 2, 0, 3, 1, 4)
        q, k, v = qkv[0], qkv[1], qkv[2]
        phi = lambda t: jnp.where(t > 0, t + 1, jnp.exp(t)) + 1e-6
        pq, pk = phi(q), phi(k)
        kv = jnp.einsum("bhsd,bhse->bhde", pk, v)
        z = jnp.einsum("bhsd->bhd", pk)
        num = jnp.einsum("bhqd,bhde->bhqe", pq, kv)
        den = jnp.einsum("bhqd,bhd->bhq", pq, z)[..., None] + 1e-6
        o = num / den
        return (lambda x, *d: x.transpose(*d))(o, 0, 2, 1, 3).reshape(B, S, D) @ wo

    def _B_ref(x, wqkv, wo):
        B, S, D = x.shape
        H = 32; Dh = D // H
        W, dil = 8, 2
        qkv = (lambda x, *d: x.transpose(*d))((x @ wqkv).reshape(B, S, 3, H, Dh), 2, 0, 3, 1, 4)
        q, k, v = qkv[0], qkv[1], qkv[2]
        scale = Dh ** -0.5
        pos = jnp.arange(S)
        off = jnp.arange(W) * dil
        idx = pos[:, None] - off[None, :]
        mask = idx >= 0
        idx_c = jnp.where(mask, idx, 0).reshape(-1)
        kg = k[:, :, idx_c, :].reshape(B, H, S, W, Dh)
        vg = v[:, :, idx_c, :].reshape(B, H, S, W, Dh)
        logits = jnp.einsum("bhsd,bhswd->bhsw", q, kg) * scale
        logits = jnp.where(mask[None, None, :, :], logits, -1e9)
        attn = _softmax(logits, axis=-1)
        o = jnp.einsum("bhsw,bhswd->bhsd", attn, vg)
        return (lambda x, *d: x.transpose(*d))(o, 0, 2, 1, 3).reshape(B, S, D) @ wo

    x = A_x
    g = _sigmoid((x * gate_w).sum(-1, keepdims=True))
    a = _A_ref(x, A_wqkv, A_wo)
    b = _B_ref(x, B_wqkv, B_wo)
    return g * a + (1 - g) * b
```

```python
import jax
import jax.numpy as jnp
from jax import lax
import jax.experimental.pallas as pl
import jax.experimental.pallas.tpu as pltpu

S, D, H, DH, W = 2048, 512, 32, 16, 8
NJ = 8
NC = S // NJ
NA = 512
F32, BF16 = jnp.float32, jnp.bfloat16
NT = (((1,), (1,)), ((), ()))


def _phi(t):
    return jnp.where(t > 0, t + 1.0, jnp.exp(t)) + 1e-6


def _kernel(x_ref, wa_ref, woa_ref, wb_ref, wob_ref, gw_ref, o_ref,
            tmp, tmp2, wka, wqa, wva_t, woa_t, wbt, wcat, xp, tacc, zacc, qb, kk, vv, ocat, xs, os_):
    def perm_t(src, dst, row0):
        t = src.astype(F32).T
        for c in range(4):
            tmp[c] = t[:, c * 128:(c + 1) * 128]
        for d in range(0, DH):
            for c in range(4):
                dst[pl.ds(row0 + d * H, H), c * 128:(c + 1) * 128] = (
                    tmp[c, pl.ds(d, H, stride=DH), :].astype(BF16))

    perm_t(wa_ref[:, D:2 * D], wka, 0)
    perm_t(wa_ref[:, 0:D], wqa, 0)
    wqa[pl.ds(D, 16), :] = jnp.broadcast_to(gw_ref[...], (16, D))
    for p in range(3):
        perm_t(wb_ref[:, p * D:(p + 1) * D], wbt, p * D)
    wva_t[...] = wa_ref[:, 2 * D:3 * D].astype(F32).T.astype(BF16)
    woa_t[...] = woa_ref[...].astype(F32).T.astype(BF16)
    for c in range(4):
        tmp[c] = wob_ref[:, c * 128:(c + 1) * 128].astype(F32)
    for d in range(DH):
        for c in range(4):
            tmp2[pl.ds(d * H, H), c * 128:(c + 1) * 128] = tmp[c, pl.ds(d, H, stride=DH), :]
    wcat[:, D:2 * D] = tmp2[...].T.astype(BF16)

    tacc[...] = jnp.zeros_like(tacc)
    zacc[...] = jnp.zeros_like(zacc)

    def s0(t, c):
        xt = x_ref[pl.ds(pl.multiple_of(t * NA, NA), NA), :]
        pk = _phi(lax.dot_general(wka[...], xt, NT, preferred_element_type=F32))
        tacc[...] += jnp.dot(pk.astype(BF16), xt, preferred_element_type=F32)
        zs = pk[:, 0:128]
        for i in range(1, NA // 128):
            zs = zs + pk[:, i * 128:(i + 1) * 128]
        zacc[...] += zs
        return c
    lax.fori_loop(0, S // NA, s0, 0)

    zacc[...] = jnp.broadcast_to(jnp.sum(zacc[...], axis=1, keepdims=True), (D, 128))
    kvt = lax.dot_general(wva_t[...], tacc[...].astype(BF16), NT, preferred_element_type=F32)
    rh = lax.broadcasted_iota(jnp.int32, (D, D), 0) // DH
    ch = lax.broadcasted_iota(jnp.int32, (D, D), 1) % H
    kvt = jnp.where(rh == ch, kvt, 0.0).astype(BF16)
    wcat[:, 0:D] = jnp.dot(woa_t[...], kvt, preferred_element_type=F32).astype(BF16)

    for c in range(4):
        xs[c] = pltpu.bitcast(x_ref[:, c * 128:(c + 1) * 128], jnp.uint32)
    x32 = xs
    o32 = os_

    def s1(j, c):
        xt = jnp.concatenate(
            [pltpu.bitcast(x32[c, pl.ds(j, NC // 2, stride=NJ), :], BF16) for c in range(4)], axis=1)
        xp[j] = xt
        qb[j] = lax.dot_general(wbt[0:D, :], xt, NT, preferred_element_type=F32) * 0.25
        k = lax.dot_general(wbt[D:2 * D, :], xt, NT, preferred_element_type=F32)
        kk[j + NJ] = k
        kk[j] = pltpu.roll(k, 2, 1)
        v = lax.dot_general(wbt[2 * D:3 * D, :], xt, NT, preferred_element_type=F32)
        vv[j + NJ] = v
        vv[j] = pltpu.roll(v, 2, 1)
        return c
    lax.fori_loop(0, NJ, s1, 0)

    lane = lax.broadcasted_iota(jnp.int32, (8, 128), 1)

    def s2(j, c):
        qa = lax.dot_general(wqa[...], xp[j], NT, preferred_element_type=F32)
        g = jax.nn.sigmoid(qa[D:D + 8, :])
        for ct in range(NC // 128):
            cs = slice(ct * 128, (ct + 1) * 128)
            gc = g[:, cs]
            for hp in range(2):
                pq, den = [], None
                for d in range(DH):
                    r = d * H + hp * 16
                    p = _phi(qa[r:r + 16, cs])
                    pq.append(p)
                    t = p * zacc[pl.ds(r, 16), :]
                    den = t if den is None else den + t
                rr = jnp.concatenate([gc, gc], axis=0) / (den + 1e-6)
                for d in range(DH):
                    ocat[pl.ds(d * H + hp * 16, 16), cs] = (pq[d] * rr).astype(BF16)
                outs = []
                for hg in range(2):
                    r0 = hp * 16 + hg * 8
                    lg = [None] * W
                    for d in range(DH):
                        rs = pl.ds(d * H + r0, 8)
                        q = qb[j, rs, cs]
                        for w in range(W):
                            t = q * kk[j + (NJ - w), rs, cs]
                            lg[w] = t if lg[w] is None else lg[w] + t
                    if ct == 0:
                        for w in range(1, W):
                            lg[w] = jnp.where(jnp.logical_and(lane < 2, j < w), -1e9, lg[w])
                    m = lg[0]
                    for w in range(1, W):
                        m = jnp.maximum(m, lg[w])
                    e = [jnp.exp(l - m) for l in lg]
                    sm = e[0]
                    for w in range(1, W):
                        sm = sm + e[w]
                    rn = (1.0 - gc) / sm
                    e = [a * rn for a in e]
                    od = []
                    for d in range(DH):
                        rs = pl.ds(d * H + r0, 8)
                        acc = None
                        for w in range(W):
                            t = e[w] * vv[j + (NJ - w), rs, cs]
                            acc = t if acc is None else acc + t
                        od.append(acc)
                    outs.append(od)
                for d in range(DH):
                    ocat[pl.ds(D + d * H + hp * 16, 16), cs] = jnp.concatenate(
                        [outs[0][d], outs[1][d]], axis=0).astype(BF16)
        ot = jnp.dot(wcat[...], ocat[...], preferred_element_type=F32)
        ob = pltpu.bitcast(ot.T.astype(BF16), jnp.uint32)
        for cc in range(4):
            o32[cc, pl.ds(j, NC // 2, stride=NJ), :] = ob[:, cc * 128:(cc + 1) * 128]
        return c
    lax.fori_loop(0, NJ, s2, 0)
    for c in range(4):
        o_ref[:, c * 128:(c + 1) * 128] = pltpu.bitcast(os_[c], BF16)


@jax.jit
def pallas_gated_mix__linear_attn_block__sliding_local_dilated__prompt_kernel(
    A_x: jax.Array,
    A_wqkv: jax.Array,
    A_wo: jax.Array,
    B_x: jax.Array,
    B_wqkv: jax.Array,
    B_wo: jax.Array,
    gate_w: jax.Array,
):
    del B_x
    out = pl.pallas_call(
        _kernel,
        out_shape=jax.ShapeDtypeStruct((S, D), BF16),
        scratch_shapes=[
            pltpu.VMEM((4, D, 128), F32),
            pltpu.VMEM((D, D), F32),
            pltpu.VMEM((D, D), BF16),
            pltpu.VMEM((D + 16, D), BF16),
            pltpu.VMEM((D, D), BF16),
            pltpu.VMEM((D, D), BF16),
            pltpu.VMEM((3 * D, D), BF16),
            pltpu.VMEM((D, 2 * D), BF16),
            pltpu.VMEM((NJ, NC, D), BF16),
            pltpu.VMEM((D, D), F32),
            pltpu.VMEM((D, 128), F32),
            pltpu.VMEM((NJ, D, NC), F32),
            pltpu.VMEM((2 * NJ, D, NC), F32),
            pltpu.VMEM((2 * NJ, D, NC), F32),
            pltpu.VMEM((2 * D, NC), BF16),
            pltpu.VMEM((4, S // 2, 128), jnp.uint32),
            pltpu.VMEM((4, S // 2, 128), jnp.uint32),
        ],
        compiler_params=pltpu.CompilerParams(vmem_limit_bytes=100 * 2**20),
    )(A_x.reshape(S, D), A_wqkv, A_wo, B_wqkv, B_wo, gate_w.reshape(1, D))
    return out.reshape(1, S, D)
```

```python
import jax
import jax.numpy as jnp
from jax import lax
import jax.experimental.pallas as pl
import jax.experimental.pallas.tpu as pltpu

S, D, H, DH, W = 2048, 512, 32, 16, 8
NJ = 8
NC = S // NJ
NA = 512
F32, BF16 = jnp.float32, jnp.bfloat16
NT = (((1,), (1,)), ((), ()))


def _phi(t):
    return jnp.where(t > 0, t + 1.0, jnp.exp(t)) + 1e-6


def _kernel(x_hbm, wa_hbm, woa_hbm, wb_hbm, wob_hbm, gw_ref, o_hbm,
            wa, woa, wb, wob, tmp, tmp2, tmp3, wka, wqa, wbt, wcat, xp, tacc, zacc,
            qb, kk, vv, gs, ocat, xs, os_, sems):
    x32 = x_hbm.bitcast(jnp.uint32)
    o32 = o_hbm.bitcast(jnp.uint32)
    RA = NA // 2
    NT0 = S // NA
    xcp = [[pltpu.make_async_copy(x32.at[pl.ds(t * RA, RA), pl.ds(c * 128, 128)],
                                  xs.at[c, pl.ds(t * RA, RA), :], sems.at[t * 4 + c])
            for c in range(4)] for t in range(NT0)],
    xcp = xcp[0]
    n0 = NT0 * 4
    wk_cp = pltpu.make_async_copy(wa_hbm.at[:, pl.ds(D, D)], wa.at[:, pl.ds(D, D)], sems.at[n0])
    wq_cp = pltpu.make_async_copy(wa_hbm.at[:, pl.ds(0, D)], wa.at[:, pl.ds(0, D)], sems.at[n0 + 1])
    wv_cp = pltpu.make_async_copy(wa_hbm.at[:, pl.ds(2 * D, D)], wa.at[:, pl.ds(2 * D, D)], sems.at[n0 + 2])
    wb_cp = pltpu.make_async_copy(wb_hbm, wb, sems.at[n0 + 3])
    woa_cp = pltpu.make_async_copy(woa_hbm, woa, sems.at[n0 + 4])
    wob_cp = pltpu.make_async_copy(wob_hbm, wob, sems.at[n0 + 5])
    wk_cp.start()
    for cp in xcp[0]:
        cp.start()
    wq_cp.start()
    for cp in xcp[1]:
        cp.start()
    wb_cp.start()
    for t in range(2, NT0):
        for cp in xcp[t]:
            cp.start()
    wob_cp.start()
    wv_cp.start()
    woa_cp.start()

    def perm_t(src, gather, dst, row0):
        t = src.astype(F32).T
        for c in range(4):
            gather[c] = t[:, c * 128:(c + 1) * 128]
        for d in range(DH):
            for c in range(4):
                dst[pl.ds(row0 + d * H, H), c * 128:(c + 1) * 128] = (
                    gather[c, pl.ds(d, H, stride=DH), :].astype(BF16))

    def perm_rows_t(gather, col0):
        for d in range(DH):
            for c in range(4):
                tmp2[pl.ds(d * H, H), c * 128:(c + 1) * 128] = gather[c, pl.ds(d, H, stride=DH), :]
        wcat[:, col0:col0 + D] = tmp2[...].T.astype(BF16)

    wk_cp.wait()
    wka[...] = wa[:, D:2 * D].astype(F32).T.astype(BF16)
    for t in range(NT0):
        for cp in xcp[t]:
            cp.wait()
        xt = jnp.concatenate(
            [pltpu.bitcast(xs[c, pl.ds(t * RA, RA), :], BF16) for c in range(4)], axis=1)
        pk = _phi(lax.dot_general(wka[...], xt, NT, preferred_element_type=F32))
        tn = jnp.dot(pk.astype(BF16), xt, preferred_element_type=F32)
        zs = pk[:, 0:128]
        for i in range(1, NA // 128):
            zs = zs + pk[:, i * 128:(i + 1) * 128]
        if t == 0:
            tacc[...] = tn
            zacc[...] = zs
            wq_cp.wait()
            perm_t(wa[:, 0:D], tmp, wqa, 0)
        else:
            tacc[...] += tn
            zacc[...] += zs
        if t == 1:
            wb_cp.wait()
            perm_t(wb[:, 0:D], tmp3, wbt, 0)
            wbt[pl.ds(3 * D, 16), :] = jnp.broadcast_to(gw_ref[...].reshape(1, D), (16, D))
        if t == 2:
            perm_t(wb[:, D:2 * D], tmp, wbt, D)
            wob_cp.wait()
            for c in range(4):
                tmp3[c] = wob[:, c * 128:(c + 1) * 128].astype(F32)
            perm_rows_t(tmp3, D)
        if t == 3:
            perm_t(wb[:, 2 * D:3 * D], tmp, wbt, 2 * D)

    wv_cp.wait()
    woa_cp.wait()
    zn = jnp.broadcast_to(jnp.sum(zacc[...], axis=1, keepdims=True), (D, 128))
    tmp3[0] = zn
    for d in range(DH):
        zacc[pl.ds(d * H, H), :] = tmp3[0, pl.ds(d, H, stride=DH), :]
    rh = lax.broadcasted_iota(jnp.int32, (128, 128), 0) // DH
    ch = lax.broadcasted_iota(jnp.int32, (128, 128), 1) // DH
    for g in range(4):
        rs = slice(g * 128, (g + 1) * 128)
        kv = jnp.dot(tacc[rs, :].astype(BF16), wa[:, 2 * D + g * 128:2 * D + (g + 1) * 128],
                     preferred_element_type=F32)
        kv = jnp.where(rh == ch, kv, 0.0).astype(BF16)
        mt = jnp.dot(kv, woa[rs, :], preferred_element_type=F32)
        for c in range(4):
            tmp[c, rs, :] = mt[:, c * 128:(c + 1) * 128]
    perm_rows_t(tmp, 0)

    ocat[...] = jnp.zeros_like(ocat)

    def s1(j, c):
        xt = jnp.concatenate(
            [pltpu.bitcast(xs[cc, pl.ds(j, NC // 2, stride=NJ), :], BF16) for cc in range(4)], axis=1)
        xp[j] = xt
        k = lax.dot_general(wbt[D:2 * D, :], xt, NT, preferred_element_type=F32)
        kk[j + NJ] = k
        kk[j] = pltpu.roll(k, 2, 1)
        v = lax.dot_general(wbt[2 * D:, :], xt, NT, preferred_element_type=F32)
        gs[j] = jax.nn.sigmoid(v[D:D + 8, :])
        v = v[:D]
        vv[j + NJ] = v
        vv[j] = pltpu.roll(v, 2, 1)
        qb[j] = lax.dot_general(wbt[0:D, :], xt, NT, preferred_element_type=F32) * 0.25
        return c
    lax.fori_loop(0, NJ, s1, 0)

    lane = lax.broadcasted_iota(jnp.int32, (8, 128), 1)

    def project(slot, jo):
        ot = jnp.dot(wcat[...], ocat[slot], preferred_element_type=F32)
        ob = pltpu.bitcast(ot.T.astype(BF16), jnp.uint32)
        for cc in range(4):
            os_[cc, pl.ds(jo, NC // 2, stride=NJ), :] = ob[:, cc * 128:(cc + 1) * 128]

    def s2(j, c):
        sl = j % 2
        project(1 - sl, (j + NJ - 1) % NJ)
        qa = lax.dot_general(wqa[...], xp[j], NT, preferred_element_type=F32)
        g = gs[j]
        for ct in range(NC // 128):
            cs = slice(ct * 128, (ct + 1) * 128)
            gc = g[:, cs]
            for hp in range(2):
                pq, den = [], None
                for d in range(DH):
                    r = d * H + hp * 16
                    p = _phi(qa[r:r + 16, cs])
                    pq.append(p)
                    t = p * zacc[pl.ds(r, 16), :]
                    den = t if den is None else den + t
                rr = jnp.concatenate([gc, gc], axis=0) / (den + 1e-6)
                for d in range(DH):
                    ocat[sl, pl.ds(d * H + hp * 16, 16), cs] = (pq[d] * rr).astype(BF16)
                outs = []
                for hg in range(2):
                    r0 = hp * 16 + hg * 8
                    lg = [None] * W
                    for d in range(DH):
                        rs = pl.ds(d * H + r0, 8)
                        q = qb[j, rs, cs]
                        for w in range(W):
                            t = q * kk[j + (NJ - w), rs, cs]
                            lg[w] = t if lg[w] is None else lg[w] + t
                    if ct == 0:
                        for w in range(1, W):
                            lg[w] = jnp.where(jnp.logical_and(lane < 2, j < w), -1e9, lg[w])
                    m = lg[0]
                    for w in range(1, W):
                        m = jnp.maximum(m, lg[w])
                    e = [jnp.exp(l - m) for l in lg]
                    sm = e[0]
                    for w in range(1, W):
                        sm = sm + e[w]
                    rn = (1.0 - gc) / sm
                    e = [a * rn for a in e]
                    od = []
                    for d in range(DH):
                        rs = pl.ds(d * H + r0, 8)
                        acc = None
                        for w in range(W):
                            t = e[w] * vv[j + (NJ - w), rs, cs]
                            acc = t if acc is None else acc + t
                        od.append(acc)
                    outs.append(od)
                for d in range(DH):
                    ocat[sl, pl.ds(D + d * H + hp * 16, 16), cs] = jnp.concatenate(
                        [outs[0][d], outs[1][d]], axis=0).astype(BF16)
        return c
    lax.fori_loop(0, NJ, s2, 0)
    project((NJ - 1) % 2, NJ - 1)
    ocp = [pltpu.make_async_copy(os_.at[c], o32.at[:, pl.ds(c * 128, 128)], sems.at[c])
           for c in range(4)]
    for cp in ocp:
        cp.start()
    for cp in ocp:
        cp.wait()


@jax.jit
def pallas_gated_mix__linear_attn_block__sliding_local_dilated__prompt_kernel(
    A_x: jax.Array,
    A_wqkv: jax.Array,
    A_wo: jax.Array,
    B_x: jax.Array,
    B_wqkv: jax.Array,
    B_wo: jax.Array,
    gate_w: jax.Array,
):
    del B_x
    out = pl.pallas_call(
        _kernel,
        out_shape=jax.ShapeDtypeStruct((S, D), BF16),
        in_specs=[pl.BlockSpec(memory_space=pl.ANY)] * 5 + [pl.BlockSpec(memory_space=pltpu.VMEM)],
        out_specs=pl.BlockSpec(memory_space=pl.ANY),
        scratch_shapes=[
            pltpu.VMEM((D, 3 * D), BF16),
            pltpu.VMEM((D, D), BF16),
            pltpu.VMEM((D, 3 * D), BF16),
            pltpu.VMEM((D, D), BF16),
            pltpu.VMEM((4, D, 128), F32),
            pltpu.VMEM((D, D), F32),
            pltpu.VMEM((4, D, 128), F32),
            pltpu.VMEM((D, D), BF16),
            pltpu.VMEM((D, D), BF16),
            pltpu.VMEM((3 * D + 16, D), BF16),
            pltpu.VMEM((D, 2 * D), BF16),
            pltpu.VMEM((NJ, NC, D), BF16),
            pltpu.VMEM((D, D), F32),
            pltpu.VMEM((D, 128), F32),
            pltpu.VMEM((NJ, D, NC), F32),
            pltpu.VMEM((2 * NJ, D, NC), F32),
            pltpu.VMEM((2 * NJ, D, NC), F32),
            pltpu.VMEM((NJ, 8, NC), F32),
            pltpu.VMEM((2, 2 * D, NC), BF16),
            pltpu.VMEM((4, S // 2, 128), jnp.uint32),
            pltpu.VMEM((4, S // 2, 128), jnp.uint32),
            pltpu.SemaphoreType.DMA((S // NA * 4 + 6,)),
        ],
        compiler_params=pltpu.CompilerParams(vmem_limit_bytes=100 * 2**20),
    )(A_x.reshape(S, D), A_wqkv, A_wo, B_wqkv, B_wo, gate_w)
    return out.reshape(1, S, D)
```

```python
import jax
import jax.numpy as jnp
from jax import lax
import jax.experimental.pallas as pl
import jax.experimental.pallas.tpu as pltpu

S, D, H, DH, W = 2048, 512, 32, 16, 8
NJ = 8
NC = S // NJ
NA = 512
F32, BF16 = jnp.float32, jnp.bfloat16
NT = (((1,), (1,)), ((), ()))


def _phi(t):
    return jnp.where(t > 0, t + 1.0, jnp.exp(t)) + 1e-6


def _kernel(x_hbm, wa_hbm, woa_hbm, wb_hbm, wob_hbm, gw_ref, o_hbm,
            wa, woa, wb, wob, tmp, tmp2, tmp3, wka, wqa, wbt, wcat, xp, tacc, zacc,
            qb, kk, vv, gs, ocat, xs, os_, sems):
    x32 = x_hbm.bitcast(jnp.uint32)
    o32 = o_hbm.bitcast(jnp.uint32)
    RA = NA // 2
    NT0 = S // NA
    xcp = [[pltpu.make_async_copy(x32.at[pl.ds(t * RA, RA), pl.ds(c * 128, 128)],
                                  xs.at[c, pl.ds(t * RA, RA), :], sems.at[t * 4 + c])
            for c in range(4)] for t in range(NT0)],
    xcp = xcp[0]
    n0 = NT0 * 4
    wk_cp = pltpu.make_async_copy(wa_hbm.at[:, pl.ds(D, D)], wa.at[:, pl.ds(D, D)], sems.at[n0])
    wq_cp = pltpu.make_async_copy(wa_hbm.at[:, pl.ds(0, D)], wa.at[:, pl.ds(0, D)], sems.at[n0 + 1])
    wv_cp = pltpu.make_async_copy(wa_hbm.at[:, pl.ds(2 * D, D)], wa.at[:, pl.ds(2 * D, D)], sems.at[n0 + 2])
    wb_cp = pltpu.make_async_copy(wb_hbm, wb, sems.at[n0 + 3])
    woa_cp = pltpu.make_async_copy(woa_hbm, woa, sems.at[n0 + 4])
    wob_cp = pltpu.make_async_copy(wob_hbm, wob, sems.at[n0 + 5])
    wk_cp.start()
    for cp in xcp[0]:
        cp.start()
    wq_cp.start()
    for cp in xcp[1]:
        cp.start()
    wb_cp.start()
    for t in range(2, NT0):
        for cp in xcp[t]:
            cp.start()
    wob_cp.start()
    wv_cp.start()
    woa_cp.start()

    def perm_t(src, gather, dst, row0):
        for c in range(4):
            gather[c] = src[c * 128:(c + 1) * 128, :].astype(F32).T
            yield
        for d in range(DH):
            for c in range(4):
                dst[pl.ds(row0 + d * H, H), c * 128:(c + 1) * 128] = (
                    gather[c, pl.ds(d, H, stride=DH), :].astype(BF16))
            if d % 4 == 3:
                yield

    def perm_rows_t(gather, col0):
        for d in range(DH):
            for c in range(4):
                tmp2[pl.ds(d * H, H), c * 128:(c + 1) * 128] = gather[c, pl.ds(d, H, stride=DH), :]
            if d % 4 == 3:
                yield
        for c in range(4):
            wcat[c * 128:(c + 1) * 128, col0:col0 + D] = (
                tmp2[:, c * 128:(c + 1) * 128].T.astype(BF16))
            yield

    def prep():
        wq_cp.wait()
        yield from perm_t(wa.at[:, pl.ds(0, D)], tmp, wqa, 0)
        wb_cp.wait()
        wbt[pl.ds(3 * D, 16), :] = jnp.broadcast_to(gw_ref[...].reshape(1, D), (16, D))
        yield from perm_t(wb.at[:, pl.ds(0, D)], tmp3, wbt, 0)
        yield from perm_t(wb.at[:, pl.ds(D, D)], tmp, wbt, D)
        yield from perm_t(wb.at[:, pl.ds(2 * D, D)], tmp3, wbt, 2 * D)
        wob_cp.wait()
        for c in range(4):
            tmp[c] = wob[:, c * 128:(c + 1) * 128].astype(F32)
        yield
        yield from perm_rows_t(tmp, D)

    pg = prep()

    def step(n):
        for _ in range(n):
            next(pg, None)

    wk_cp.wait()
    wka[...] = wa[:, D:2 * D].astype(F32).T.astype(BF16)
    MH = 256
    for t in range(NT0):
        for cp in xcp[t]:
            cp.wait()
        xt = jnp.concatenate(
            [pltpu.bitcast(xs[c, pl.ds(t * RA, RA), :], BF16) for c in range(4)], axis=1)
        for m in range(D // MH):
            rs = slice(m * MH, (m + 1) * MH)
            pk = _phi(lax.dot_general(wka[rs, :], xt, NT, preferred_element_type=F32))
            step(3)
            tn = jnp.dot(pk.astype(BF16), xt, preferred_element_type=F32)
            zs = pk[:, 0:128]
            for i in range(1, NA // 128):
                zs = zs + pk[:, i * 128:(i + 1) * 128]
            if t == 0:
                tacc[rs, :] = tn
                zacc[rs, :] = zs
            else:
                tacc[rs, :] += tn
                zacc[rs, :] += zs
            step(3)
    step(100)

    wv_cp.wait()
    woa_cp.wait()
    zn = jnp.broadcast_to(jnp.sum(zacc[...], axis=1, keepdims=True), (D, 128))
    tmp3[0] = zn
    for d in range(DH):
        zacc[pl.ds(d * H, H), :] = tmp3[0, pl.ds(d, H, stride=DH), :]
    rh = lax.broadcasted_iota(jnp.int32, (128, 128), 0) // DH
    ch = lax.broadcasted_iota(jnp.int32, (128, 128), 1) // DH
    for g in range(4):
        rs = slice(g * 128, (g + 1) * 128)
        kv = jnp.dot(tacc[rs, :].astype(BF16), wa[:, 2 * D + g * 128:2 * D + (g + 1) * 128],
                     preferred_element_type=F32)
        kv = jnp.where(rh == ch, kv, 0.0).astype(BF16)
        mt = jnp.dot(kv, woa[rs, :], preferred_element_type=F32)
        for c in range(4):
            tmp[c, rs, :] = mt[:, c * 128:(c + 1) * 128]
    for _ in perm_rows_t(tmp, 0):
        pass

    ocat[...] = jnp.zeros_like(ocat)

    def s1(j, c):
        xt = jnp.concatenate(
            [pltpu.bitcast(xs[cc, pl.ds(j, NC // 2, stride=NJ), :], BF16) for cc in range(4)], axis=1)
        xp[j] = xt
        k = lax.dot_general(wbt[D:2 * D, :], xt, NT, preferred_element_type=F32)
        kk[j + NJ] = k
        kk[j] = pltpu.roll(k, 2, 1)
        v = lax.dot_general(wbt[2 * D:, :], xt, NT, preferred_element_type=F32)
        gs[j] = jax.nn.sigmoid(v[D:D + 8, :])
        v = v[:D]
        vv[j + NJ] = v
        vv[j] = pltpu.roll(v, 2, 1)
        qb[j] = lax.dot_general(wbt[0:D, :], xt, NT, preferred_element_type=F32) * 0.25
        return c
    lax.fori_loop(0, NJ, s1, 0)

    lane = lax.broadcasted_iota(jnp.int32, (8, 128), 1)

    def piece(slot, jo, i):
        ot = jnp.dot(wcat[i * 128:(i + 1) * 128, :], ocat[slot], preferred_element_type=F32)
        os_[i, pl.ds(jo, NC // 2, stride=NJ), :] = pltpu.bitcast(ot.T.astype(BF16), jnp.uint32)

    def s2(j, c):
        sl = j % 2
        jo = (j + NJ - 1) % NJ
        qa = lax.dot_general(wqa[...], xp[j], NT, preferred_element_type=F32)
        g = gs[j]
        ot = jnp.dot(wcat[...], ocat[1 - sl], preferred_element_type=F32)

        def side_a(ct, hp):
            cs = slice(ct * 128, (ct + 1) * 128)
            gc = g[:, cs]
            pq, den = [], None
            for d in range(DH):
                r = d * H + hp * 16
                p = _phi(qa[r:r + 16, cs])
                pq.append(p)
                t = p * zacc[pl.ds(r, 16), :]
                den = t if den is None else den + t
            rr = jnp.concatenate([gc, gc], axis=0) / (den + 1e-6)
            for d in range(DH):
                ocat[sl, pl.ds(d * H + hp * 16, 16), cs] = (pq[d] * rr).astype(BF16)

        def side_b(ct, hp):
            cs = slice(ct * 128, (ct + 1) * 128)
            gc = g[:, cs]
            outs = []
            for hg in range(2):
                r0 = hp * 16 + hg * 8
                lg = [None] * W
                for d in range(DH):
                    rs = pl.ds(d * H + r0, 8)
                    q = qb[j, rs, cs]
                    for w in range(W):
                        t = q * kk[j + (NJ - w), rs, cs]
                        lg[w] = t if lg[w] is None else lg[w] + t
                if ct == 0:
                    for w in range(1, W):
                        lg[w] = jnp.where(jnp.logical_and(lane < 2, j < w), -1e9, lg[w])
                m = lg[0]
                for w in range(1, W):
                    m = jnp.maximum(m, lg[w])
                e = [jnp.exp(l - m) for l in lg]
                sm = e[0]
                for w in range(1, W):
                    sm = sm + e[w]
                rn = (1.0 - gc) / sm
                e = [a * rn for a in e]
                od = []
                for d in range(DH):
                    rs = pl.ds(d * H + r0, 8)
                    acc = None
                    for w in range(W):
                        t = e[w] * vv[j + (NJ - w), rs, cs]
                        acc = t if acc is None else acc + t
                    od.append(acc)
                outs.append(od)
            for d in range(DH):
                ocat[sl, pl.ds(D + d * H + hp * 16, 16), cs] = jnp.concatenate(
                    [outs[0][d], outs[1][d]], axis=0).astype(BF16)

        for i, (ct, hp) in enumerate([(0, 0), (0, 1), (1, 0), (1, 1)]):
            side_b(ct, hp)
            side_a(ct, hp)
        ob = pltpu.bitcast(ot.T.astype(BF16), jnp.uint32)
        for i in range(4):
            os_[i, pl.ds(jo, NC // 2, stride=NJ), :] = ob[:, i * 128:(i + 1) * 128]
        return c
    lax.fori_loop(0, NJ, s2, 0)
    for i in range(4):
        piece((NJ - 1) % 2, NJ - 1, i)
    ocp = [pltpu.make_async_copy(os_.at[c], o32.at[:, pl.ds(c * 128, 128)], sems.at[c])
           for c in range(4)]
    for cp in ocp:
        cp.start()
    for cp in ocp:
        cp.wait()


@jax.jit
def pallas_gated_mix__linear_attn_block__sliding_local_dilated__prompt_kernel(
    A_x: jax.Array,
    A_wqkv: jax.Array,
    A_wo: jax.Array,
    B_x: jax.Array,
    B_wqkv: jax.Array,
    B_wo: jax.Array,
    gate_w: jax.Array,
):
    del B_x
    out = pl.pallas_call(
        _kernel,
        out_shape=jax.ShapeDtypeStruct((S, D), BF16),
        in_specs=[pl.BlockSpec(memory_space=pl.ANY)] * 5 + [pl.BlockSpec(memory_space=pltpu.VMEM)],
        out_specs=pl.BlockSpec(memory_space=pl.ANY),
        scratch_shapes=[
            pltpu.VMEM((D, 3 * D), BF16),
            pltpu.VMEM((D, D), BF16),
            pltpu.VMEM((D, 3 * D), BF16),
            pltpu.VMEM((D, D), BF16),
            pltpu.VMEM((4, D, 128), F32),
            pltpu.VMEM((D, D), F32),
            pltpu.VMEM((4, D, 128), F32),
            pltpu.VMEM((D, D), BF16),
            pltpu.VMEM((D, D), BF16),
            pltpu.VMEM((3 * D + 16, D), BF16),
            pltpu.VMEM((D, 2 * D), BF16),
            pltpu.VMEM((NJ, NC, D), BF16),
            pltpu.VMEM((D, D), F32),
            pltpu.VMEM((D, 128), F32),
            pltpu.VMEM((NJ, D, NC), F32),
            pltpu.VMEM((2 * NJ, D, NC), F32),
            pltpu.VMEM((2 * NJ, D, NC), F32),
            pltpu.VMEM((NJ, 8, NC), F32),
            pltpu.VMEM((2, 2 * D, NC), BF16),
            pltpu.VMEM((4, S // 2, 128), jnp.uint32),
            pltpu.VMEM((4, S // 2, 128), jnp.uint32),
            pltpu.SemaphoreType.DMA((S // NA * 4 + 6,)),
        ],
        compiler_params=pltpu.CompilerParams(vmem_limit_bytes=100 * 2**20),
    )(A_x.reshape(S, D), A_wqkv, A_wo, B_wqkv, B_wo, gate_w)
    return out.reshape(1, S, D)
```

```python
import jax
import jax.numpy as jnp
from jax import lax
import jax.experimental.pallas as pl
import jax.experimental.pallas.tpu as pltpu

S, D, H, DH, W = 2048, 512, 32, 16, 8
NJ = 8
NC = S // NJ
NA = 512
F32, BF16 = jnp.float32, jnp.bfloat16
NT = (((1,), (1,)), ((), ()))


def _phi(t):
    return jnp.where(t > 0, t + 1.0, jnp.exp(t)) + 1e-6


def _kernel(x_hbm, wa_hbm, woa_hbm, wb_hbm, wob_hbm, gw_ref, o_hbm,
            wa, woa, wb, wob, tmp, tmp2, tmp3, wka, wqa, wbt, wcat, tacc, zacc,
            qb, kk, vv, gs, ocat, xs, os_, sems):
    x32 = x_hbm.bitcast(jnp.uint32)
    o32 = o_hbm.bitcast(jnp.uint32)
    RA = NA // 2
    NT0 = S // NA
    xcp = [[pltpu.make_async_copy(x32.at[pl.ds(t * RA, RA), pl.ds(c * 128, 128)],
                                  xs.at[c, pl.ds(t * RA, RA), :], sems.at[t * 4 + c])
            for c in range(4)] for t in range(NT0)],
    xcp = xcp[0]
    n0 = NT0 * 4
    wk_cp = pltpu.make_async_copy(wa_hbm.at[:, pl.ds(D, D)], wa.at[:, pl.ds(D, D)], sems.at[n0])
    wq_cp = pltpu.make_async_copy(wa_hbm.at[:, pl.ds(0, D)], wa.at[:, pl.ds(0, D)], sems.at[n0 + 1])
    wv_cp = pltpu.make_async_copy(wa_hbm.at[:, pl.ds(2 * D, D)], wa.at[:, pl.ds(2 * D, D)], sems.at[n0 + 2])
    wb_cp = pltpu.make_async_copy(wb_hbm, wb, sems.at[n0 + 3])
    woa_cp = pltpu.make_async_copy(woa_hbm, woa, sems.at[n0 + 4])
    wob_cp = pltpu.make_async_copy(wob_hbm, wob, sems.at[n0 + 5])
    wk_cp.start()
    for cp in xcp[0]:
        cp.start()
    wq_cp.start()
    for cp in xcp[1]:
        cp.start()
    wb_cp.start()
    for t in range(2, NT0):
        for cp in xcp[t]:
            cp.start()
    wob_cp.start()
    wv_cp.start()
    woa_cp.start()

    def perm_t(src, gather, dst, row0):
        for c in range(4):
            gather[c] = src[c * 128:(c + 1) * 128, :].astype(F32).T
            yield
        for d in range(DH):
            for c in range(4):
                dst[pl.ds(row0 + d * H, H), c * 128:(c + 1) * 128] = (
                    gather[c, pl.ds(d, H, stride=DH), :].astype(BF16))
            if d % 4 == 3:
                yield

    def perm_rows_t(gather, col0):
        for d in range(DH):
            for c in range(4):
                tmp2[pl.ds(d * H, H), c * 128:(c + 1) * 128] = gather[c, pl.ds(d, H, stride=DH), :]
            if d % 4 == 3:
                yield
        for c in range(4):
            wcat[c * 128:(c + 1) * 128, col0:col0 + D] = (
                tmp2[:, c * 128:(c + 1) * 128].T.astype(BF16))
            yield

    def prep():
        wq_cp.wait()
        yield from perm_t(wa.at[:, pl.ds(0, D)], tmp, wqa, 0)
        wb_cp.wait()
        wbt[pl.ds(3 * D, 16), :] = jnp.broadcast_to(gw_ref[...].reshape(1, D), (16, D))
        yield from perm_t(wb.at[:, pl.ds(0, D)], tmp3, wbt, 0)
        yield from perm_t(wb.at[:, pl.ds(D, D)], tmp, wbt, D)
        yield from perm_t(wb.at[:, pl.ds(2 * D, D)], tmp3, wbt, 2 * D)
        wob_cp.wait()
        for c in range(4):
            tmp[c] = wob[:, c * 128:(c + 1) * 128].astype(F32)
        yield
        yield from perm_rows_t(tmp, D)

    pg = prep()

    def step(n):
        for _ in range(n):
            next(pg, None)

    wk_cp.wait()
    wka[...] = wa[:, D:2 * D].astype(F32).T.astype(BF16)
    MH = 256
    for t in range(NT0):
        for cp in xcp[t]:
            cp.wait()
        xt = jnp.concatenate(
            [pltpu.bitcast(xs[c, pl.ds(t * RA, RA), :], BF16) for c in range(4)], axis=1)
        for m in range(D // MH):
            rs = slice(m * MH, (m + 1) * MH)
            pk = _phi(lax.dot_general(wka[rs, :], xt, NT, preferred_element_type=F32))
            step(3)
            tn = jnp.dot(pk.astype(BF16), xt, preferred_element_type=F32)
            zs = pk[:, 0:128]
            for i in range(1, NA // 128):
                zs = zs + pk[:, i * 128:(i + 1) * 128]
            if t == 0:
                tacc[rs, :] = tn
                zacc[rs, :] = zs
            else:
                tacc[rs, :] += tn
                zacc[rs, :] += zs
            step(3)
    step(100)

    wv_cp.wait()
    woa_cp.wait()
    zn = jnp.broadcast_to(jnp.sum(zacc[...], axis=1, keepdims=True), (D, 128))
    tmp3[0] = zn
    for d in range(DH):
        zacc[pl.ds(d * H, H), :] = tmp3[0, pl.ds(d, H, stride=DH), :]
    rh = lax.broadcasted_iota(jnp.int32, (128, 128), 0) // DH
    ch = lax.broadcasted_iota(jnp.int32, (128, 128), 1) // DH
    for g in range(4):
        rs = slice(g * 128, (g + 1) * 128)
        kv = jnp.dot(tacc[rs, :].astype(BF16), wa[:, 2 * D + g * 128:2 * D + (g + 1) * 128],
                     preferred_element_type=F32)
        kv = jnp.where(rh == ch, kv, 0.0).astype(BF16)
        mt = jnp.dot(kv, woa[rs, :], preferred_element_type=F32)
        for c in range(4):
            tmp[c, rs, :] = mt[:, c * 128:(c + 1) * 128]
    for _ in perm_rows_t(tmp, 0):
        pass

    ocat[NJ - 1] = jnp.zeros((2 * D, NC), BF16)

    def s1(j, c):
        xt = jnp.concatenate(
            [pltpu.bitcast(xs[cc, pl.ds(j, NC // 2, stride=NJ), :], BF16) for cc in range(4)], axis=1)
        k = lax.dot_general(wbt[D:2 * D, :], xt, NT, preferred_element_type=F32)
        kk[j + NJ] = k
        kk[j] = pltpu.roll(k, 2, 1)
        v = lax.dot_general(wbt[2 * D:, :], xt, NT, preferred_element_type=F32)
        g = jax.nn.sigmoid(v[D:D + 8, :])
        gs[j] = g
        qa = lax.dot_general(wqa[...], xt, NT, preferred_element_type=F32)
        v = v[:D]
        vv[j + NJ] = v
        vv[j] = pltpu.roll(v, 2, 1)
        qb[j] = lax.dot_general(wbt[0:D, :], xt, NT, preferred_element_type=F32) * 0.25

        def side_a(ct, hp):
            cs = slice(ct * 128, (ct + 1) * 128)
            gc = g[:, cs]
            pq, den = [], None
            for d in range(DH):
                r = d * H + hp * 16
                p = _phi(qa[r:r + 16, cs])
                pq.append(p)
                t = p * zacc[pl.ds(r, 16), :]
                den = t if den is None else den + t
            rr = jnp.concatenate([gc, gc], axis=0) / (den + 1e-6)
            for d in range(DH):
                ocat[j, pl.ds(d * H + hp * 16, 16), cs] = (pq[d] * rr).astype(BF16)

        for ct in range(2):
            for hp in range(2):
                side_a(ct, hp)
        return c
    lax.fori_loop(0, NJ, s1, 0)

    lane = lax.broadcasted_iota(jnp.int32, (8, 128), 1)

    def piece(slot, jo, i):
        ot = jnp.dot(wcat[i * 128:(i + 1) * 128, :], ocat[slot], preferred_element_type=F32)
        os_[i, pl.ds(jo, NC // 2, stride=NJ), :] = pltpu.bitcast(ot.T.astype(BF16), jnp.uint32)

    def s2(j, c):
        jo = (j + NJ - 1) % NJ
        g = gs[j]
        ot = jnp.dot(wcat[...], ocat[jo], preferred_element_type=F32)

        def side_b(ct, hp):
            cs = slice(ct * 128, (ct + 1) * 128)
            gc = g[:, cs]
            outs = []
            for hg in range(2):
                r0 = hp * 16 + hg * 8
                lg = [None] * W
                for d in range(DH):
                    rs = pl.ds(d * H + r0, 8)
                    q = qb[j, rs, cs]
                    for w in range(W):
                        t = q * kk[j + (NJ - w), rs, cs]
                        lg[w] = t if lg[w] is None else lg[w] + t
                if ct == 0:
                    for w in range(1, W):
                        lg[w] = jnp.where(jnp.logical_and(lane < 2, j < w), -1e9, lg[w])
                m = lg[0]
                for w in range(1, W):
                    m = jnp.maximum(m, lg[w])
                e = [jnp.exp(l - m) for l in lg]
                sm = e[0]
                for w in range(1, W):
                    sm = sm + e[w]
                rn = (1.0 - gc) / sm
                e = [a * rn for a in e]
                od = []
                for d in range(DH):
                    rs = pl.ds(d * H + r0, 8)
                    acc = None
                    for w in range(W):
                        t = e[w] * vv[j + (NJ - w), rs, cs]
                        acc = t if acc is None else acc + t
                    od.append(acc)
                outs.append(od)
            for d in range(DH):
                ocat[j, pl.ds(D + d * H + hp * 16, 16), cs] = jnp.concatenate(
                    [outs[0][d], outs[1][d]], axis=0).astype(BF16)

        for i, (ct, hp) in enumerate([(0, 0), (0, 1), (1, 0), (1, 1)]):
            side_b(ct, hp)
        ob = pltpu.bitcast(ot.T.astype(BF16), jnp.uint32)
        for i in range(4):
            os_[i, pl.ds(jo, NC // 2, stride=NJ), :] = ob[:, i * 128:(i + 1) * 128]
        return c
    lax.fori_loop(0, NJ, s2, 0)
    for i in range(4):
        piece(NJ - 1, NJ - 1, i)
    ocp = [pltpu.make_async_copy(os_.at[c], o32.at[:, pl.ds(c * 128, 128)], sems.at[c])
           for c in range(4)]
    for cp in ocp:
        cp.start()
    for cp in ocp:
        cp.wait()


@jax.jit
def pallas_gated_mix__linear_attn_block__sliding_local_dilated__prompt_kernel(
    A_x: jax.Array,
    A_wqkv: jax.Array,
    A_wo: jax.Array,
    B_x: jax.Array,
    B_wqkv: jax.Array,
    B_wo: jax.Array,
    gate_w: jax.Array,
):
    del B_x
    out = pl.pallas_call(
        _kernel,
        out_shape=jax.ShapeDtypeStruct((S, D), BF16),
        in_specs=[pl.BlockSpec(memory_space=pl.ANY)] * 5 + [pl.BlockSpec(memory_space=pltpu.VMEM)],
        out_specs=pl.BlockSpec(memory_space=pl.ANY),
        scratch_shapes=[
            pltpu.VMEM((D, 3 * D), BF16),
            pltpu.VMEM((D, D), BF16),
            pltpu.VMEM((D, 3 * D), BF16),
            pltpu.VMEM((D, D), BF16),
            pltpu.VMEM((4, D, 128), F32),
            pltpu.VMEM((D, D), F32),
            pltpu.VMEM((4, D, 128), F32),
            pltpu.VMEM((D, D), BF16),
            pltpu.VMEM((D, D), BF16),
            pltpu.VMEM((3 * D + 16, D), BF16),
            pltpu.VMEM((D, 2 * D), BF16),
            pltpu.VMEM((D, D), F32),
            pltpu.VMEM((D, 128), F32),
            pltpu.VMEM((NJ, D, NC), F32),
            pltpu.VMEM((2 * NJ, D, NC), F32),
            pltpu.VMEM((2 * NJ, D, NC), F32),
            pltpu.VMEM((NJ, 8, NC), F32),
            pltpu.VMEM((NJ, 2 * D, NC), BF16),
            pltpu.VMEM((4, S // 2, 128), jnp.uint32),
            pltpu.VMEM((4, S // 2, 128), jnp.uint32),
            pltpu.SemaphoreType.DMA((S // NA * 4 + 6,)),
        ],
        compiler_params=pltpu.CompilerParams(vmem_limit_bytes=100 * 2**20, flags={"XLA_TPU_RESCHEDULE_DMA_DONES": True}),
    )(A_x.reshape(S, D), A_wqkv, A_wo, B_wqkv, B_wo, gate_w)
    return out.reshape(1, S, D)
```
